```python
import jax
import jax.numpy as jnp

def _softmax(x, axis=-1):
    return jax.nn.softmax(x, axis=axis)
def _gelu(x):
    return jax.nn.gelu(x, approximate=True)
def _silu(x):
    return jax.nn.silu(x)
def _sigmoid(x):
    return jax.nn.sigmoid(x)
def _layernorm(x, axis=-1, eps=1e-5):
    m = jnp.mean(x, axis=axis, keepdims=True)
    v = jnp.var(x, axis=axis, keepdims=True)
    return (x - m) / jnp.sqrt(v + eps)
def _scatter_add(tgt, idx, src, axis=0):
    return tgt.at[idx].add(src)
def _segment_sum(src, seg, n):
    return jax.ops.segment_sum(src, seg, n)
class _Rng:
    def __init__(self, key):
        self._k = key
    def _next(self):
        self._k, sub = jax.random.split(self._k)
        return sub
    def normal(self, shape):
        return jax.random.normal(self._next(), shape, dtype=jnp.bfloat16)
    def randint(self, lo, hi, shape):
        return jax.random.randint(self._next(), shape, lo, hi, dtype=jnp.int32)
    def uniform(self, shape, lo=0.0, hi=1.0):
        return jax.random.uniform(self._next(), shape, jnp.bfloat16, lo, hi)
    def permutation(self, n):
        return jax.random.permutation(self._next(), n)


kernel_name = 'sequential_preLN__sliding_block_cached__glu_gated_swiglu__decode'

def setup_inputs():
    _rng = _Rng(jax.random.key(int.from_bytes(__import__("os").urandom(4), "little")))
    _w = (lambda a: (lambda t: t.astype(jnp.bfloat16) if jnp.issubdtype(t.dtype, jnp.floating) else t)(jnp.asarray(a)))
    def _A_setup():
        B, Sq, D = 1, 1, 640
        Hq, Hkv, Sk, Dh = 32, 32, 32768, 192
        assert Hq % Hkv == 0, (Hq, Hkv)
        return {
            "x": _w((lambda *s: _rng.normal(s) * 0.05)(B, Sq, D)),
            "k_cache": _w((lambda *s: _rng.normal(s) * 0.05)(B, Hkv, Sk, Dh)),
            "v_cache": _w((lambda *s: _rng.normal(s) * 0.05)(B, Hkv, Sk, Dh)),
            "wq": _w((lambda *s: _rng.normal(s) * 0.05)(D, Hq * Dh) * (D ** -0.5)),
            "wo": _w((lambda *s: _rng.normal(s) * 0.05)(Hq * Dh, D) * ((Hq * Dh) ** -0.5)),
        }
    _A_in = _A_setup()

    def _B_setup():
        B, S, D, F = 1, 1, 640, 1536
        return {
            "x": _w((lambda *s: _rng.normal(s) * 0.05)(B, S, D)),
            "w1": _w((lambda *s: _rng.normal(s) * 0.05)(D, F) * (2.0 / D) ** 0.5),
            "w3": _w((lambda *s: _rng.normal(s) * 0.05)(D, F) * (2.0 / D) ** 0.5),
            "w2": _w((lambda *s: _rng.normal(s) * 0.05)(F, D) * (2.0 / F) ** 0.5),
        }
    _B_in = _B_setup()

    return {
        "A_x": _A_in["x"],
        "A_k_cache": _A_in["k_cache"],
        "A_v_cache": _A_in["v_cache"],
        "A_wq": _A_in["wq"],
        "A_wo": _A_in["wo"],
        "B_x": _B_in["x"],
        "B_w1": _B_in["w1"],
        "B_w3": _B_in["w3"],
        "B_w2": _B_in["w2"],
    }

def reference(A_x, A_k_cache, A_v_cache, A_wq, A_wo, B_x, B_w1, B_w3, B_w2):
    def _A_ref(x, k_cache, v_cache, wq, wo):
        B, Sq, D = x.shape
        Hq, Dh = 32, 192
        Hkv, Sk = k_cache.shape[1], k_cache.shape[2]
        W = min(4096, max(256, Sk // 4))
        rep = Hq // Hkv
        q = (lambda x, *d: x.transpose(*d))((x @ wq).reshape(B, Sq, Hq, Dh), 0, 2, 1, 3)
        k = jnp.repeat(k_cache[:, :, Sk - W:, :], rep, axis=1)
        v = jnp.repeat(v_cache[:, :, Sk - W:, :], rep, axis=1)
        scores = jnp.einsum("bhqd,bhkd->bhqk", q, k) * (Dh ** -0.5)
        p = _softmax(scores, axis=-1)
        o = jnp.einsum("bhqk,bhkd->bhqd", p, v)
        return (lambda x, *d: x.transpose(*d))(o, 0, 2, 1, 3).reshape(B, Sq, Hq * Dh) @ wo

    def _B_ref(x, w1, w3, w2):
        gate = jnp.einsum("bsd,df->bsf", x, w1)
        up = jnp.einsum("bsd,df->bsf", x, w3)
        h = _silu(gate) * up
        out = jnp.einsum("bsf,fd->bsd", h, w2)
        return out

    x = A_x
    h = x + _A_ref(_layernorm(x, axis=-1), A_k_cache, A_v_cache, A_wq, A_wo)
    h2 = h + _B_ref(_layernorm(h, axis=-1), B_w1, B_w3, B_w2)
    return h2
```

```python
import functools
import jax
import jax.numpy as jnp
from jax import lax
import jax.experimental.pallas as pl
import jax.experimental.pallas.tpu as pltpu

H, DH, SK, W, D, F = 32, 192, 32768, 4096, 640, 1536
f32, bf16 = jnp.float32, jnp.bfloat16

def _ln(x, eps=1e-5):
    m = jnp.mean(x, axis=-1, keepdims=True)
    v = jnp.mean((x - m) * (x - m), axis=-1, keepdims=True)
    return (x - m) / jnp.sqrt(v + eps)

NB = 3

def kern(x_hbm, k_hbm, v_hbm, wq_hbm, wo_hbm, w1_hbm, w3_hbm, w2_hbm, o_ref,
         x_v, wq_v, kbuf, vbuf, wobuf, w1_v, w3_v, w2_v, q_scr, sem_w, sem_kv):
    def head_copies(h, slot):
        return (
            pltpu.make_async_copy(k_hbm.at[h, :, pl.ds(SK - W, W)], kbuf.at[slot], sem_kv.at[0, slot]),
            pltpu.make_async_copy(v_hbm.at[h, :, pl.ds(SK - W, W)], vbuf.at[slot], sem_kv.at[1, slot]),
            pltpu.make_async_copy(wo_hbm.at[h], wobuf.at[slot], sem_kv.at[2, slot]),
        )
    cp_x = pltpu.make_async_copy(x_hbm, x_v, sem_w.at[0])
    cp_wq = pltpu.make_async_copy(wq_hbm, wq_v, sem_w.at[1])
    cp_w1 = pltpu.make_async_copy(w1_hbm, w1_v, sem_w.at[2])
    cp_w3 = pltpu.make_async_copy(w3_hbm, w3_v, sem_w.at[3])
    cp_w2 = pltpu.make_async_copy(w2_hbm, w2_v, sem_w.at[4])
    cp_x.start()
    cp_wq.start()
    for h in range(NB):
        for c in head_copies(h, h):
            c.start()
    cp_x.wait()
    xf = x_v[...].astype(f32)
    xn = _ln(xf)
    xn8 = jnp.broadcast_to(xn, (8, D)).astype(bf16)
    cp_wq.wait()
    scale = DH ** -0.5
    for j in range(H // 2):
        q2 = jnp.dot(xn8, wq_v[:, j * 384:(j + 1) * 384], preferred_element_type=f32) * scale
        q_scr[2 * j] = q2[:, :DH].astype(bf16)
        q_scr[2 * j + 1] = q2[:, DH:].astype(bf16)

    def body(h, acc):
        slot = h % NB
        ck, cv, cwo = head_copies(h, slot)
        ck.wait()
        s = jnp.dot(q_scr[h], kbuf[slot], preferred_element_type=f32)
        m = jnp.max(s, axis=-1, keepdims=True)
        p = jnp.exp(s - m)
        l = jnp.sum(p, axis=-1, keepdims=True)
        cv.wait()
        o = lax.dot_general(p.astype(bf16), vbuf[slot], (((1,), (1,)), ((), ())), preferred_element_type=f32)
        o = o / l
        cwo.wait()
        acc = acc + jnp.dot(o.astype(bf16), wobuf[slot], preferred_element_type=f32)
        @pl.when(h + NB < H)
        def _():
            for c in head_copies(h + NB, slot):
                c.start()
        @pl.when(h + NB == H)
        def _():
            cp_w1.start()
            cp_w3.start()
        @pl.when(h + NB == H + 1)
        def _():
            cp_w2.start()
        return acc
    acc = lax.fori_loop(0, H, body, jnp.zeros((8, D), f32))
    hres = xf + acc[0:1]
    hn = _ln(hres)
    hn8 = jnp.broadcast_to(hn, (8, D)).astype(bf16)
    cp_w1.wait()
    gate = jnp.dot(hn8, w1_v[...], preferred_element_type=f32)
    cp_w3.wait()
    up = jnp.dot(hn8, w3_v[...], preferred_element_type=f32)
    hh = (gate * jax.nn.sigmoid(gate) * up).astype(bf16)
    cp_w2.wait()
    out = jnp.dot(hh, w2_v[...], preferred_element_type=f32)
    o_ref[...] = (hres + out[0:1]).astype(bf16)


@jax.jit
def pallas_sequential_preLN__sliding_block_cached__glu_gated_swiglu__decode_kernel(
    A_x: jax.Array,
    A_k_cache: jax.Array,
    A_v_cache: jax.Array,
    A_wq: jax.Array,
    A_wo: jax.Array,
    B_x: jax.Array,
    B_w1: jax.Array,
    B_w3: jax.Array,
    B_w2: jax.Array,
):
    kT = jnp.transpose(A_k_cache.reshape(H, SK, DH), (0, 2, 1))
    vT = jnp.transpose(A_v_cache.reshape(H, SK, DH), (0, 2, 1))
    anyspec = pl.BlockSpec(memory_space=pl.ANY)
    out = pl.pallas_call(
        kern, name="decode_block",
        out_shape=jax.ShapeDtypeStruct((1, D), bf16),
        in_specs=[anyspec] * 8,
        out_specs=pl.BlockSpec(memory_space=pltpu.VMEM),
        scratch_shapes=[
            pltpu.VMEM((1, D), bf16),
            pltpu.VMEM((D, H * DH), bf16),
            pltpu.VMEM((NB, DH, W), bf16),
            pltpu.VMEM((NB, DH, W), bf16),
            pltpu.VMEM((NB, DH, D), bf16),
            pltpu.VMEM((D, F), bf16),
            pltpu.VMEM((D, F), bf16),
            pltpu.VMEM((F, D), bf16),
            pltpu.VMEM((H, 8, DH), bf16),
            pltpu.SemaphoreType.DMA((5,)),
            pltpu.SemaphoreType.DMA((3, NB)),
        ],
        compiler_params=pltpu.CompilerParams(vmem_limit_bytes=100 * 1024 * 1024),
    )(A_x.reshape(1, D), kT, vT, A_wq, A_wo.reshape(H, DH, D), B_w1, B_w3, B_w2)
    return out.reshape(1, 1, D)
```

```python
import functools, contextlib
import jax
import jax.numpy as jnp
from jax import lax
import jax.experimental.pallas as pl
import jax.experimental.pallas.tpu as pltpu

H, DH, SK, W, D, F = 32, 192, 32768, 4096, 640, 1536
f32, bf16 = jnp.float32, jnp.bfloat16

def _ln(x, eps=1e-5):
    m = jnp.mean(x, axis=-1, keepdims=True)
    v = jnp.mean((x - m) * (x - m), axis=-1, keepdims=True)
    return (x - m) / jnp.sqrt(v + eps)

def make(name="kv2", NB=3, W2B=256, scopes=False):
    sc = (lambda n: jax.named_scope(n)) if scopes else (lambda n: contextlib.nullcontext())
    W2A = F - W2B
    def kern(x_hbm, k_hbm, v_hbm, wq_hbm, wo_hbm, w1_hbm, w3_hbm, w2_hbm, o_ref,
             x_v, wq_v, kbuf, vbuf, wobuf, w1_v, w3_v, w2_v, q_scr, sem_w, sem_kv):
        def head_copies(h, slot):
            return (
                pltpu.make_async_copy(k_hbm.at[h, :, pl.ds(SK - W, W)], kbuf.at[slot], sem_kv.at[0, slot]),
                pltpu.make_async_copy(v_hbm.at[h, :, pl.ds(SK - W, W)], vbuf.at[slot], sem_kv.at[1, slot]),
                pltpu.make_async_copy(wo_hbm.at[h], wobuf.at[slot], sem_kv.at[2, slot]),
            )
        cp_x = pltpu.make_async_copy(x_hbm, x_v, sem_w.at[0])
        cp_wq = pltpu.make_async_copy(wq_hbm, wq_v, sem_w.at[1])
        cp_w1 = pltpu.make_async_copy(w1_hbm, w1_v, sem_w.at[2])
        cp_w3 = pltpu.make_async_copy(w3_hbm, w3_v, sem_w.at[3])
        cp_w2a = pltpu.make_async_copy(w2_hbm.at[pl.ds(0, W2A)], w2_v.at[pl.ds(0, W2A)], sem_w.at[4])
        cp_w2b = pltpu.make_async_copy(w2_hbm.at[pl.ds(W2A, W2B)], w2_v.at[pl.ds(W2A, W2B)], sem_w.at[5])
        cp_x.start()
        cp_wq.start()
        @pl.loop(0, NB)
        def _(h):
            for c in head_copies(h, h):
                c.start()
        with sc("wX"):
            cp_x.wait()
        xf = x_v[...].astype(f32)
        xn = _ln(xf)
        xn8 = jnp.broadcast_to(xn, (8, D)).astype(bf16)
        with sc("wWq"):
            cp_wq.wait()
        scale = DH ** -0.5
        for j in range(H // 2):
            q2 = jnp.dot(xn8, wq_v[:, j * 384:(j + 1) * 384], preferred_element_type=f32) * scale
            q_scr[2 * j] = q2[:, :DH].astype(bf16)
            q_scr[2 * j + 1] = q2[:, DH:].astype(bf16)

        def body(h, acc):
            slot = h % NB
            ck, cv, cwo = head_copies(h, slot)
            with sc("wK"):
                ck.wait()
            s = jnp.dot(q_scr[h], kbuf[slot], preferred_element_type=f32)
            m = jnp.max(s, axis=-1, keepdims=True)
            p = jnp.exp(s - m)
            l = jnp.sum(p, axis=-1, keepdims=True)
            with sc("wV"):
                cv.wait()
            o = lax.dot_general(p.astype(bf16), vbuf[slot], (((1,), (1,)), ((), ())), preferred_element_type=f32)
            o = o / l
            with sc("wWo"):
                cwo.wait()
            acc = acc + jnp.dot(o.astype(bf16), wobuf[slot], preferred_element_type=f32)
            @pl.when(h + NB < H)
            def _():
                for c in head_copies(h + NB, slot):
                    c.start()
            @pl.when(h == H - 3)
            def _():
                cp_w1.start()
                cp_w3.start()
            @pl.when(h == H - 2)
            def _():
                cp_w2a.start()
            @pl.when(h == H - 1)
            def _():
                cp_w2b.start()
            return acc
        acc = lax.fori_loop(0, H, body, jnp.zeros((8, D), f32))
        hres = xf + acc[0:1]
        hn = _ln(hres)
        hn8 = jnp.broadcast_to(hn, (8, D)).astype(bf16)
        with sc("wW1"):
            cp_w1.wait()
        gate = jnp.dot(hn8, w1_v[...], preferred_element_type=f32)
        with sc("wW3"):
            cp_w3.wait()
        up = jnp.dot(hn8, w3_v[...], preferred_element_type=f32)
        hh = (gate * jax.nn.sigmoid(gate) * up).astype(bf16)
        with sc("wW2a"):
            cp_w2a.wait()
        out = jnp.dot(hh[:, :W2A], w2_v[pl.ds(0, W2A), :], preferred_element_type=f32)
        part = hres + out[0:1]
        with sc("wW2b"):
            cp_w2b.wait()
        out2 = jnp.dot(hh[:, W2A:], w2_v[pl.ds(W2A, W2B), :], preferred_element_type=f32)
        o_ref[...] = (part + out2[0:1]).astype(bf16)

    def fn(A_x, k, v, wq, wo, B_x, w1, w3, w2):
        kT = jnp.transpose(k.reshape(H, SK, DH), (0, 2, 1))
        vT = jnp.transpose(v.reshape(H, SK, DH), (0, 2, 1))
        anyspec = pl.BlockSpec(memory_space=pl.ANY)
        out = pl.pallas_call(
            kern, name=name,
            out_shape=jax.ShapeDtypeStruct((1, D), bf16),
            in_specs=[anyspec] * 8,
            out_specs=pl.BlockSpec(memory_space=pltpu.VMEM),
            scratch_shapes=[
                pltpu.VMEM((1, D), bf16),
                pltpu.VMEM((D, H * DH), bf16),
                pltpu.VMEM((NB, DH, W), bf16),
                pltpu.VMEM((NB, DH, W), bf16),
                pltpu.VMEM((NB, DH, D), bf16),
                pltpu.VMEM((D, F), bf16),
                pltpu.VMEM((D, F), bf16),
                pltpu.VMEM((F, D), bf16),
                pltpu.VMEM((H, 8, DH), bf16),
                pltpu.SemaphoreType.DMA((6,)),
                pltpu.SemaphoreType.DMA((3, NB)),
            ],
            compiler_params=pltpu.CompilerParams(vmem_limit_bytes=100 * 1024 * 1024),
        )(A_x.reshape(1, D), kT, vT, wq, wo.reshape(H, DH, D), w1, w3, w2)
        return out.reshape(1, 1, D)
    return fn


_impl = make(name="decode_block", NB=2, W2B=256)


@jax.jit
def pallas_sequential_preLN__sliding_block_cached__glu_gated_swiglu__decode_kernel(
    A_x: jax.Array,
    A_k_cache: jax.Array,
    A_v_cache: jax.Array,
    A_wq: jax.Array,
    A_wo: jax.Array,
    B_x: jax.Array,
    B_w1: jax.Array,
    B_w3: jax.Array,
    B_w2: jax.Array,
):
    return _impl(A_x, A_k_cache, A_v_cache, A_wq, A_wo, B_x, B_w1, B_w3, B_w2)
```

```python
import functools, contextlib
import jax
import jax.numpy as jnp
from jax import lax
import jax.experimental.pallas as pl
import jax.experimental.pallas.tpu as pltpu

H, DH, SK, W, D, F = 32, 192, 32768, 4096, 640, 1536
f32, bf16 = jnp.float32, jnp.bfloat16

def _ln(x, eps=1e-5):
    m = jnp.mean(x, axis=-1, keepdims=True)
    v = jnp.mean((x - m) * (x - m), axis=-1, keepdims=True)
    return (x - m) / jnp.sqrt(v + eps)

def make(name="kv6", w13mode="alt", ffn_loop=False, qloop=False, NB=2, W2B=240, scopes=False, CS=2048, QCS=2048, WOR=24, W13R=8, W2R=24, dbc=True,
         kvorder="il", pro_heads=1):
    sc = (lambda n: jax.named_scope(n)) if scopes else (lambda n: contextlib.nullcontext())
    W2A = F - W2B
    def kern(x_hbm, k_hbm, v_hbm, wq_hbm, wo_hbm, w1_hbm, w3_hbm, w2_hbm, o_ref,
             x_v, wq_v, kbuf, vbuf, wobuf, w1_v, w3_v, w2_v, q_scr, sem_w, sem_kv):

        def start_alt(pairs):
            for n, (src, dst, sem) in enumerate(pairs):
                pltpu.make_async_copy(src, dst, sem).start(priority=n % 2)

        def start_head(h, slot):
            pieces = [(r, c) for r in range(0, DH, 8) for c in range(0, W, CS)]
            kp = [(k_hbm.at[h, pl.ds(r, 8), pl.ds(SK - W + c, CS)], kbuf.at[slot, pl.ds(r, 8), pl.ds(c, CS)], sem_kv.at[0, slot]) for r, c in pieces]
            vp = [(v_hbm.at[h, pl.ds(r, 8), pl.ds(SK - W + c, CS)], vbuf.at[slot, pl.ds(r, 8), pl.ds(c, CS)], sem_kv.at[1, slot]) for r, c in pieces]
            wp = [(wo_hbm.at[h, pl.ds(r, WOR)], wobuf.at[slot, pl.ds(r, WOR)], sem_kv.at[2, slot]) for r in range(0, DH, WOR)]
            if kvorder == "il":
                seq = [t for pr in zip(kp, vp) for t in pr] + wp
            else:
                seq = kp + vp + wp
            start_alt(seq)

        def wait_all(buf, sem):
            pltpu.make_async_copy(buf, buf, sem).wait()

        cp_x = pltpu.make_async_copy(x_hbm, x_v, sem_w.at[0])
        cp_x.start()
        @pl.loop(0, D // 16)
        def _(i):
            seq = []
            for rr in (0, 8):
                r = pl.multiple_of(i * 16 + rr, 8)
                for c in range(0, H * DH, QCS):
                    seq.append((wq_hbm.at[pl.ds(r, 8), pl.ds(c, QCS)], wq_v.at[pl.ds(r, 8), pl.ds(c, QCS)], sem_w.at[1]))
            start_alt(seq)
        for h in range(pro_heads):
            start_head(h, h)
        with sc("wX"):
            cp_x.wait()
        xf = x_v[...].astype(f32)
        xn = _ln(xf)
        xn8 = jnp.broadcast_to(xn, (8, D)).astype(bf16)
        with sc("wWq"):
            wait_all(wq_v, sem_w.at[1])
        scale = DH ** -0.5
        if qloop:
            @pl.loop(0, H // 2)
            def _(j):
                c = pl.multiple_of(j * 384, 128)
                q2 = jnp.dot(xn8, wq_v[:, pl.ds(c, 384)], preferred_element_type=f32) * scale
                q_scr[2 * j] = q2[:, :DH].astype(bf16)
                q_scr[2 * j + 1] = q2[:, DH:].astype(bf16)
        else:
            for j in range(H // 2):
                q2 = jnp.dot(xn8, wq_v[:, j * 384:(j + 1) * 384], preferred_element_type=f32) * scale
                q_scr[2 * j] = q2[:, :DH].astype(bf16)
                q_scr[2 * j + 1] = q2[:, DH:].astype(bf16)
        @pl.loop(pro_heads, NB)
        def _(h):
            start_head(h, h)

        def body(h, acc):
            slot = h % NB
            with sc("wK"):
                wait_all(kbuf.at[slot], sem_kv.at[0, slot])
            s = jnp.dot(q_scr[h], kbuf[slot], preferred_element_type=f32)
            m = jnp.max(s, axis=-1, keepdims=True)
            p = jnp.exp(s - m)
            l = jnp.sum(p, axis=-1, keepdims=True)
            with sc("wV"):
                wait_all(vbuf.at[slot], sem_kv.at[1, slot])
            o = lax.dot_general(p.astype(bf16), vbuf[slot], (((1,), (1,)), ((), ())), preferred_element_type=f32)
            o = o / l
            with sc("wWo"):
                wait_all(wobuf.at[slot], sem_kv.at[2, slot])
            acc = acc + jnp.dot(o.astype(bf16), wobuf[slot], preferred_element_type=f32)
            with sc("issue"):
                @pl.when(h + NB < H)
                def _():
                    start_head(h + NB, slot)
                @pl.when(h + NB == H)
                def _():
                    a1 = [(w1_hbm.at[pl.ds(r, W13R)], w1_v.at[pl.ds(r, W13R)], sem_w.at[2]) for r in range(0, D, W13R)]
                    a3 = [(w3_hbm.at[pl.ds(r, W13R)], w3_v.at[pl.ds(r, W13R)], sem_w.at[3]) for r in range(0, D, W13R)]
                    if w13mode == "il":
                        seq = [t for pr in zip(a1, a3) for t in pr]
                    elif w13mode == "alt":
                        seq = a1 + a3
                    elif w13mode == "alt2":
                        seq = [t for i in range(0, len(a1), 2) for t in (a1[i], a1[i+1], a3[i], a3[i+1])]
                    start_alt(seq)
                @pl.when(h == H - 1)
                def _():
                    seq = [(w2_hbm.at[pl.ds(r, W2R)], w2_v.at[pl.ds(r, W2R)], sem_w.at[4 if r < W2A else 5]) for r in range(0, F, W2R)]
                    start_alt(seq)
            return acc
        acc = lax.fori_loop(0, H, body, jnp.zeros((8, D), f32))
        hres = xf + acc[0:1]
        hn = _ln(hres)
        hn8 = jnp.broadcast_to(hn, (8, D)).astype(bf16)
        with sc("wW1"):
            wait_all(w1_v, sem_w.at[2])
        gate = jnp.dot(hn8, w1_v[...], preferred_element_type=f32)
        with sc("wW3"):
            wait_all(w3_v, sem_w.at[3])
        up = jnp.dot(hn8, w3_v[...], preferred_element_type=f32)
        hh = (gate * jax.nn.sigmoid(gate) * up).astype(bf16)
        with sc("wW2a"):
            wait_all(w2_v.at[pl.ds(0, W2A)], sem_w.at[4])
        out = jnp.dot(hh[:, :W2A], w2_v[pl.ds(0, W2A), :], preferred_element_type=f32)
        part = hres + out[0:1]
        with sc("wW2b"):
            wait_all(w2_v.at[pl.ds(W2A, W2B)], sem_w.at[5])
        out2 = jnp.dot(hh[:, W2A:], w2_v[pl.ds(W2A, W2B), :], preferred_element_type=f32)
        o_ref[...] = (part + out2[0:1]).astype(bf16)

    def fn(A_x, k, v, wq, wo, B_x, w1, w3, w2):
        kT = jnp.transpose(k.reshape(H, SK, DH), (0, 2, 1))
        vT = jnp.transpose(v.reshape(H, SK, DH), (0, 2, 1))
        anyspec = pl.BlockSpec(memory_space=pl.ANY)
        out = pl.pallas_call(
            kern, name=name,
            out_shape=jax.ShapeDtypeStruct((1, D), bf16),
            in_specs=[anyspec] * 8,
            out_specs=pl.BlockSpec(memory_space=pltpu.VMEM),
            scratch_shapes=[
                pltpu.VMEM((1, D), bf16),
                pltpu.VMEM((D, H * DH), bf16),
                pltpu.VMEM((NB, DH, W), bf16),
                pltpu.VMEM((NB, DH, W), bf16),
                pltpu.VMEM((NB, DH, D), bf16),
                pltpu.VMEM((D, F), bf16),
                pltpu.VMEM((D, F), bf16),
                pltpu.VMEM((F, D), bf16),
                pltpu.VMEM((H, 8, DH), bf16),
                pltpu.SemaphoreType.DMA((6,)),
                pltpu.SemaphoreType.DMA((3, NB)),
            ],
            compiler_params=pltpu.CompilerParams(vmem_limit_bytes=100 * 1024 * 1024, disable_bounds_checks=dbc),
        )(A_x.reshape(1, D), kT, vT, wq, wo.reshape(H, DH, D), w1, w3, w2)
        return out.reshape(1, 1, D)
    return fn


_impl = make(name="decode_block", NB=2, W2B=384, w13mode='alt', kvorder='kv')


@jax.jit
def pallas_sequential_preLN__sliding_block_cached__glu_gated_swiglu__decode_kernel(
    A_x: jax.Array,
    A_k_cache: jax.Array,
    A_v_cache: jax.Array,
    A_wq: jax.Array,
    A_wo: jax.Array,
    B_x: jax.Array,
    B_w1: jax.Array,
    B_w3: jax.Array,
    B_w2: jax.Array,
):
    return _impl(A_x, A_k_cache, A_v_cache, A_wq, A_wo, B_x, B_w1, B_w3, B_w2)
```

```python
import functools, contextlib
import jax
import jax.numpy as jnp
from jax import lax
import jax.experimental.pallas as pl
import jax.experimental.pallas.tpu as pltpu

H, DH, SK, W, D, F = 32, 192, 32768, 4096, 640, 1536
f32, bf16 = jnp.float32, jnp.bfloat16

def _ln(x, eps=1e-5):
    m = jnp.mean(x, axis=-1, keepdims=True)
    v = jnp.mean((x - m) * (x - m), axis=-1, keepdims=True)
    return (x - m) / jnp.sqrt(v + eps)

def make(name="kv8", scopes=False, CS=2048, QCS=2048, WOR=24, W13R=8,
         kvorder="cm", wq_stride=16, wq_grp=2, wo_stride=16, wo_grp=1, w13streams=4, w13mode="il",
         w2chunks=(1152, 256, 128), w2rows=16, w2streams0=1,
         wopos="early", issue_pos="afterpv", it13=H - 2, it2=H - 1):
    NB = 2
    sc = (lambda n: jax.named_scope(n)) if scopes else (lambda n: contextlib.nullcontext())
    assert sum(w2chunks) == F and len(w2chunks) <= 3
    w2off = [sum(w2chunks[:i]) for i in range(len(w2chunks))]
    NQ = (D // 8) * (H * DH // QCS)
    NO = H * DH // WOR
    def kern(x_hbm, k_hbm, v_hbm, wq_hbm, wo_hbm, w1_hbm, w3_hbm, w2_hbm, o_ref,
             x_v, wq_v, wo_v, kbuf, vbuf, w1_v, w3_v, w2_v, q_scr, sem):
        def start_alt(pairs, first=0):
            for n, (src, dst, s) in enumerate(pairs):
                pltpu.make_async_copy(src, dst, s).start(priority=(n + first) % 2)

        def start_head(h, slot):
            if kvorder == "cm":
                pieces = [(r, c) for c in range(0, W, CS) for r in range(0, DH, 8)]
            else:
                pieces = [(r, c) for r in range(0, DH, 8) for c in range(0, W, CS)]
            kp = [(k_hbm.at[h, pl.ds(r, 8), pl.ds(SK - W + c, CS)], kbuf.at[slot, pl.ds(r, 8), pl.ds(c, CS)], sem.at[slot]) for r, c in pieces]
            vp = [(v_hbm.at[h, pl.ds(r, 8), pl.ds(SK - W + c, CS)], vbuf.at[slot, pl.ds(r, 8), pl.ds(c, CS)], sem.at[2 + slot]) for r, c in pieces]
            start_alt(kp + vp)

        def wait_all(buf, s):
            pltpu.make_async_copy(buf, buf, s).wait()

        cp_x = pltpu.make_async_copy(x_hbm, x_v, sem.at[3])
        cp_x.start()
        ncb = H * DH // QCS
        @pl.loop(0, wq_stride // wq_grp)
        def _(it):
            seq = []
            for b in range(NQ // wq_stride):
                for i in range(wq_grp):
                    p = wq_stride * b + i + wq_grp * it
                    r = lax.div(p, ncb)
                    c = p - ncb * r
                    r8 = pl.multiple_of(r * 8, 8)
                    cc = pl.multiple_of(c * QCS, QCS)
                    seq.append((wq_hbm.at[pl.ds(r8, 8), pl.ds(cc, QCS)], wq_v.at[pl.ds(r8, 8), pl.ds(cc, QCS)], sem.at[1]))
            start_alt(seq)

        def start_wo(s):
            @pl.loop(0, wo_stride // wo_grp)
            def _(it):
                seq = []
                for b in range(NO // wo_stride):
                    for i in range(wo_grp):
                        p = wo_stride * b + i + wo_grp * it
                        r = pl.multiple_of(p * WOR, 8)
                        seq.append((wo_hbm.at[pl.ds(r, WOR)], wo_v.at[pl.ds(r, WOR)], s))
                start_alt(seq)
        if wopos == "early":
            start_wo(sem.at[1])
        start_head(0, 0)
        with sc("wX"):
            cp_x.wait()
        xf = x_v[...].astype(f32)
        xn = _ln(xf)
        xn8 = jnp.broadcast_to(xn, (8, D)).astype(bf16)
        with sc("wWq"):
            wait_all(wq_v, sem.at[1])
            if wopos == "early":
                wait_all(wo_v, sem.at[1])
        start_head(1, 1)
        scale = DH ** -0.5
        with sc("qcomp"):
            for j in range(H // 2):
                q2 = jnp.dot(xn8, wq_v[:, j * 384:(j + 1) * 384], preferred_element_type=f32) * scale
                q_scr[2 * j] = q2[:, :DH].astype(bf16)
                q_scr[2 * j + 1] = q2[:, DH:].astype(bf16)
        if wopos == "late":
            start_wo(sem.at[4])

        def start_w13():
            nrg = D // W13R
            per = nrg // w13streams
            order = [(i % w13streams) * per + i // w13streams for i in range(nrg)]
            a1 = [(w1_hbm.at[pl.ds(g * W13R, W13R)], w1_v.at[pl.ds(g * W13R, W13R)], sem.at[0]) for g in order]
            a3 = [(w3_hbm.at[pl.ds(g * W13R, W13R)], w3_v.at[pl.ds(g * W13R, W13R)], sem.at[2]) for g in order]
            if w13mode == "il":
                seq = [t for pr in zip(a1, a3) for t in pr]
            else:
                seq = a1 + a3
            start_alt(seq)

        w2sems = [1, 3, 4]
        def w2piece(r, n):
            ci = max(i for i, o in enumerate(w2off) if o <= r)
            assert r + n <= w2off[ci] + w2chunks[ci], (r, n)
            return (w2_hbm.at[pl.ds(r, n)], w2_v.at[pl.ds(r, n)], sem.at[w2sems[ci]])

        def start_w2():
            ra = list(range(0, F // 2, w2rows))
            if w2streams0 > 1:
                per = len(ra) // w2streams0
                ra = [ra[(i % w2streams0) * per + i // w2streams0] for i in range(len(ra))]
            a = [w2piece(r, w2rows) for r in ra]
            b = [w2piece(r, w2rows) for r in range(F // 2, F, w2rows)]
            start_alt([t for pr in zip(a, b) for t in pr])

        def issue(h, slot):
            with sc("issue"):
                @pl.when(h + NB < H)
                def _():
                    start_head(h + NB, slot)
                @pl.when(h == it13)
                def _():
                    start_w13()
                @pl.when(h == it2)
                def _():
                    start_w2()

        def body(h, acc):
            slot = h % NB
            with sc("wK"):
                wait_all(kbuf.at[slot], sem.at[slot])
            s = jnp.dot(q_scr[h], kbuf[slot], preferred_element_type=f32)
            m = jnp.max(s, axis=-1, keepdims=True)
            p = jnp.exp(s - m)
            l = jnp.sum(p, axis=-1, keepdims=True)
            with sc("wV"):
                wait_all(vbuf.at[slot], sem.at[2 + slot])
            o = lax.dot_general(p.astype(bf16), vbuf[slot], (((1,), (1,)), ((), ())), preferred_element_type=f32)
            o = o / l
            if issue_pos == "afterpv":
                issue(h, slot)
            if wopos == "late":
                @pl.when(h == 0)
                def _():
                    wait_all(wo_v, sem.at[4])
            r0 = pl.multiple_of(h * DH, 64)
            acc = acc + jnp.dot(o.astype(bf16), wo_v[pl.ds(r0, DH), :], preferred_element_type=f32)
            if issue_pos == "end":
                issue(h, slot)
            return acc
        acc = lax.fori_loop(0, H, body, jnp.zeros((8, D), f32))
        hres = xf + acc[0:1]
        hn = _ln(hres)
        hn8 = jnp.broadcast_to(hn, (8, D)).astype(bf16)
        with sc("wW1"):
            wait_all(w1_v, sem.at[0])
        gate = jnp.dot(hn8, w1_v[...], preferred_element_type=f32)
        with sc("wW3"):
            wait_all(w3_v, sem.at[2])
        up = jnp.dot(hn8, w3_v[...], preferred_element_type=f32)
        hh = (gate * jax.nn.sigmoid(gate) * up).astype(bf16)
        part = hres
        for ci, (o, n) in enumerate(zip(w2off, w2chunks)):
            with sc(f"wW2_{ci}"):
                wait_all(w2_v.at[pl.ds(o, n)], sem.at[w2sems[ci]])
            out = jnp.dot(hh[:, o:o + n], w2_v[pl.ds(o, n), :], preferred_element_type=f32)
            part = part + out[0:1]
        o_ref[...] = part.astype(bf16)

    def fn(A_x, k, v, wq, wo, B_x, w1, w3, w2):
        kT = jnp.transpose(k.reshape(H, SK, DH), (0, 2, 1))
        vT = jnp.transpose(v.reshape(H, SK, DH), (0, 2, 1))
        anyspec = pl.BlockSpec(memory_space=pl.ANY)
        out = pl.pallas_call(
            kern, name=name,
            out_shape=jax.ShapeDtypeStruct((1, D), bf16),
            in_specs=[anyspec] * 8,
            out_specs=pl.BlockSpec(memory_space=pltpu.VMEM),
            scratch_shapes=[
                pltpu.VMEM((1, D), bf16),
                pltpu.VMEM((D, H * DH), bf16),
                pltpu.VMEM((H * DH, D), bf16),
                pltpu.VMEM((NB, DH, W), bf16),
                pltpu.VMEM((NB, DH, W), bf16),
                pltpu.VMEM((D, F), bf16),
                pltpu.VMEM((D, F), bf16),
                pltpu.VMEM((F, D), bf16),
                pltpu.VMEM((H, 8, DH), bf16),
                pltpu.SemaphoreType.DMA((5,)),
            ],
            compiler_params=pltpu.CompilerParams(vmem_limit_bytes=100 * 1024 * 1024, disable_bounds_checks=True),
        )(A_x.reshape(1, D), kT, vT, wq, wo, w1, w3, w2)
        return out.reshape(1, 1, D)
    return fn


_impl = make(name="decode_block", )


@jax.jit
def pallas_sequential_preLN__sliding_block_cached__glu_gated_swiglu__decode_kernel(
    A_x: jax.Array,
    A_k_cache: jax.Array,
    A_v_cache: jax.Array,
    A_wq: jax.Array,
    A_wo: jax.Array,
    B_x: jax.Array,
    B_w1: jax.Array,
    B_w3: jax.Array,
    B_w2: jax.Array,
):
    return _impl(A_x, A_k_cache, A_v_cache, A_wq, A_wo, B_x, B_w1, B_w3, B_w2)
```

```python
import jax
import jax.numpy as jnp
from jax import lax
import jax.experimental.pallas as pl
import jax.experimental.pallas.tpu as pltpu

H, DH, SK, D, F = 32, 192, 32768, 640, 1536
W = min(4096, max(256, SK // 4))
HD = H * DH
EPS = 1e-5
f32, bf16 = jnp.float32, jnp.bfloat16

LANES = 2048
WO_ROWS = 24
W13_ROWS = 8
W2_ROWS = 16
W2_CHUNKS = ((0, 1152, 1), (1152, 256, 3), (1408, 128, 4))


def _layernorm(x):
    m = jnp.mean(x, axis=-1, keepdims=True)
    v = jnp.mean((x - m) * (x - m), axis=-1, keepdims=True)
    return (x - m) / jnp.sqrt(v + EPS)


def _start_alternating(copies):
    for n, (src, dst, sem) in enumerate(copies):
        pltpu.make_async_copy(src, dst, sem).start(priority=n % 2)


def _wait_filled(buf, sem):
    pltpu.make_async_copy(buf, buf, sem).wait()


def _kernel(x_hbm, k_hbm, v_hbm, wq_hbm, wo_hbm, w1_hbm, w3_hbm, w2_hbm, o_ref,
            x_v, wq_v, wo_v, kbuf, vbuf, w1_v, w3_v, w2_v, q_scr, sem):

    def start_head(h, slot):
        pieces = [(r, c) for c in range(0, W, LANES) for r in range(0, DH, 8)]
        copies = []
        for src, dst, s in ((k_hbm, kbuf, sem.at[slot]), (v_hbm, vbuf, sem.at[2 + slot])):
            copies += [(src.at[h, pl.ds(r, 8), pl.ds(SK - W + c, LANES)],
                        dst.at[slot, pl.ds(r, 8), pl.ds(c, LANES)], s) for r, c in pieces]
        _start_alternating(copies)

    x_copy = pltpu.make_async_copy(x_hbm, x_v, sem.at[3])
    x_copy.start()

    ncb = HD // LANES
    n_wq = (D // 8) * ncb

    @pl.loop(0, 8)
    def _(it):
        copies = []
        for b in range(n_wq // 16):
            for i in range(2):
                p = 16 * b + i + 2 * it
                r = lax.div(p, ncb)
                rows = pl.ds(pl.multiple_of(r * 8, 8), 8)
                cols = pl.ds(pl.multiple_of((p - ncb * r) * LANES, LANES), LANES)
                copies.append((wq_hbm.at[rows, cols], wq_v.at[rows, cols], sem.at[1]))
        _start_alternating(copies)

    n_wo = HD // WO_ROWS

    @pl.loop(0, 16)
    def _(it):
        copies = []
        for b in range(n_wo // 16):
            rows = pl.ds(pl.multiple_of((16 * b + it) * WO_ROWS, 8), WO_ROWS)
            copies.append((wo_hbm.at[rows], wo_v.at[rows], sem.at[4]))
        _start_alternating(copies)

    start_head(0, 0)

    x_copy.wait()
    xf = x_v[...].astype(f32)
    xn = jnp.broadcast_to(_layernorm(xf), (8, D)).astype(bf16)
    _wait_filled(wq_v, sem.at[1])
    start_head(1, 1)

    scale = DH ** -0.5
    for j in range(H // 2):
        q2 = jnp.dot(xn, wq_v[:, j * 2 * DH:(j + 1) * 2 * DH],
                     preferred_element_type=f32) * scale
        q_scr[2 * j] = q2[:, :DH].astype(bf16)
        q_scr[2 * j + 1] = q2[:, DH:].astype(bf16)
    _wait_filled(wo_v, sem.at[4])

    def start_w1_w3():
        groups = D // W13_ROWS
        copies = []
        for i in range(groups):
            g = (i % 4) * (groups // 4) + i // 4
            rows = pl.ds(g * W13_ROWS, W13_ROWS)
            copies.append((w1_hbm.at[rows], w1_v.at[rows], sem.at[0]))
            copies.append((w3_hbm.at[rows], w3_v.at[rows], sem.at[2]))
        _start_alternating(copies)

    def start_w2():
        def piece(r):
            s = [sm for off, n, sm in W2_CHUNKS if off <= r < off + n][0]
            rows = pl.ds(r, W2_ROWS)
            return (w2_hbm.at[rows], w2_v.at[rows], sem.at[s])
        copies = []
        for r in range(0, F // 2, W2_ROWS):
            copies += [piece(r), piece(r + F // 2)]
        _start_alternating(copies)

    def head(h, acc):
        slot = h % 2
        _wait_filled(kbuf.at[slot], sem.at[slot])
        s = jnp.dot(q_scr[h], kbuf[slot], preferred_element_type=f32)
        m = jnp.max(s, axis=-1, keepdims=True)
        p = jnp.exp(s - m)
        l = jnp.sum(p, axis=-1, keepdims=True)
        _wait_filled(vbuf.at[slot], sem.at[2 + slot])
        o = lax.dot_general(p.astype(bf16), vbuf[slot], (((1,), (1,)), ((), ())),
                            preferred_element_type=f32) / l

        @pl.when(h + 2 < H)
        def _():
            start_head(h + 2, slot)

        @pl.when(h == H - 2)
        def _():
            start_w1_w3()

        @pl.when(h == H - 1)
        def _():
            start_w2()

        rows = pl.ds(pl.multiple_of(h * DH, 64), DH)
        return acc + jnp.dot(o.astype(bf16), wo_v[rows, :], preferred_element_type=f32)

    attn = lax.fori_loop(0, H, head, jnp.zeros((8, D), f32))
    h1 = xf + attn[0:1]

    hn = jnp.broadcast_to(_layernorm(h1), (8, D)).astype(bf16)
    _wait_filled(w1_v, sem.at[0])
    gate = jnp.dot(hn, w1_v[...], preferred_element_type=f32)
    _wait_filled(w3_v, sem.at[2])
    up = jnp.dot(hn, w3_v[...], preferred_element_type=f32)
    act = (gate * jax.nn.sigmoid(gate) * up).astype(bf16)

    out = h1
    for off, n, s in W2_CHUNKS:
        _wait_filled(w2_v.at[pl.ds(off, n)], sem.at[s])
        part = jnp.dot(act[:, off:off + n], w2_v[pl.ds(off, n), :],
                       preferred_element_type=f32)
        out = out + part[0:1]
    o_ref[...] = out.astype(bf16)


@jax.jit
def pallas_sequential_preLN__sliding_block_cached__glu_gated_swiglu__decode_kernel(
    A_x: jax.Array,
    A_k_cache: jax.Array,
    A_v_cache: jax.Array,
    A_wq: jax.Array,
    A_wo: jax.Array,
    B_x: jax.Array,
    B_w1: jax.Array,
    B_w3: jax.Array,
    B_w2: jax.Array,
):
    del B_x
    k_t = jnp.transpose(A_k_cache.reshape(H, SK, DH), (0, 2, 1))
    v_t = jnp.transpose(A_v_cache.reshape(H, SK, DH), (0, 2, 1))
    hbm = pl.BlockSpec(memory_space=pl.ANY)
    out = pl.pallas_call(
        _kernel,
        name="decode_block",
        out_shape=jax.ShapeDtypeStruct((1, D), bf16),
        in_specs=[hbm] * 8,
        out_specs=pl.BlockSpec(memory_space=pltpu.VMEM),
        scratch_shapes=[
            pltpu.VMEM((1, D), bf16),
            pltpu.VMEM((D, HD), bf16),
            pltpu.VMEM((HD, D), bf16),
            pltpu.VMEM((2, DH, W), bf16),
            pltpu.VMEM((2, DH, W), bf16),
            pltpu.VMEM((D, F), bf16),
            pltpu.VMEM((D, F), bf16),
            pltpu.VMEM((F, D), bf16),
            pltpu.VMEM((H, 8, DH), bf16),
            pltpu.SemaphoreType.DMA((5,)),
        ],
        compiler_params=pltpu.CompilerParams(vmem_limit_bytes=64 * 1024 * 1024),
    )(A_x.reshape(1, D), k_t, v_t, A_wq, A_wo, B_w1, B_w3, B_w2)
    return out.reshape(1, 1, D)
```
